```python
import os as _os
_os.environ.setdefault("JAX_PLATFORMS", "cpu")
import jax
import jax.numpy as jnp

def _softmax(x, axis=-1):
    return jax.nn.softmax(x, axis=axis)
def _gelu(x):
    return jax.nn.gelu(x, approximate=True)
def _silu(x):
    return jax.nn.silu(x)
def _sigmoid(x):
    return jax.nn.sigmoid(x)
def _layernorm(x, axis=-1, eps=1e-5):
    m = jnp.mean(x, axis=axis, keepdims=True)
    v = jnp.var(x, axis=axis, keepdims=True)
    return (x - m) / jnp.sqrt(v + eps)
def _scatter_add(tgt, idx, src, axis=0):
    return tgt.at[idx].add(src)
def _segment_sum(src, seg, n):
    return jax.ops.segment_sum(src, seg, n)
class _Rng:
    def __init__(self, key):
        self._k = key
    def _next(self):
        self._k, sub = jax.random.split(self._k)
        return sub
    def normal(self, shape):
        return jax.random.normal(self._next(), shape, dtype=jnp.bfloat16)
    def randint(self, lo, hi, shape):
        return jax.random.randint(self._next(), shape, lo, hi, dtype=jnp.int32)
    def uniform(self, shape, lo=0.0, hi=1.0):
        return jax.random.uniform(self._next(), shape, jnp.bfloat16, lo, hi)
    def permutation(self, n):
        return jax.random.permutation(self._next(), n)


kernel_name = 'concat_heads__gqa_block_cached__mha_block_cached__near_ridge'

def setup_inputs():
    _rng = _Rng(jax.random.key(int.from_bytes(__import__("os").urandom(4), "little")))
    _w = (lambda a: (lambda t: t.astype(jnp.bfloat16) if jnp.issubdtype(t.dtype, jnp.floating) else t)(jnp.asarray(a)))
    def _A_setup():
        B, Sq, D = 16, 32, 512
        Hq, Hkv, Sk, Dh = 32, 8, 512, 128
        assert Hq % Hkv == 0, (Hq, Hkv)
        return {
            "x": _w((lambda *s: _rng.normal(s) * 0.8)(B, Sq, D)),
            "k_cache": _w((lambda *s: _rng.normal(s) * 0.8)(B, Hkv, Sk, Dh)),
            "v_cache": _w((lambda *s: _rng.normal(s) * 0.05)(B, Hkv, Sk, Dh)),
            "wq": _w((lambda *s: _rng.normal(s) * 0.8)(D, Hq * Dh) * (D ** -0.5)),
            "wo": _w((lambda *s: _rng.normal(s) * 0.05)(Hq * Dh, D) * ((Hq * Dh) ** -0.5)),
        }
    _A_in = _A_setup()

    def _B_setup():
        B, Sq, D = 16, 32, 512
        H, Sk, Dh = 32, 512, 128
        return {
            "x": _w((lambda *s: _rng.normal(s) * 0.8)(B, Sq, D)),
            "k_cache": _w((lambda *s: _rng.normal(s) * 0.8)(B, H, Sk, Dh)),
            "v_cache": _w((lambda *s: _rng.normal(s) * 0.05)(B, H, Sk, Dh)),
            "wq": _w((lambda *s: _rng.normal(s) * 0.8)(D, H * Dh) * (D ** -0.5)),
            "wo": _w((lambda *s: _rng.normal(s) * 0.05)(H * Dh, D) * ((H * Dh) ** -0.5)),
        }
    _B_in = _B_setup()

    return {
        "A_x": _A_in["x"],
        "A_k_cache": _A_in["k_cache"],
        "A_v_cache": _A_in["v_cache"],
        "A_wq": _A_in["wq"],
        "A_wo": _A_in["wo"],
        "B_x": _B_in["x"],
        "B_k_cache": _B_in["k_cache"],
        "B_v_cache": _B_in["v_cache"],
        "B_wq": _B_in["wq"],
        "B_wo": _B_in["wo"],
    }

def reference(A_x, A_k_cache, A_v_cache, A_wq, A_wo, B_x, B_k_cache, B_v_cache, B_wq, B_wo):
    def _A_ref(x, k_cache, v_cache, wq, wo):
        B, Sq, D = x.shape
        Hq, Dh = 32, 128
        Hkv = k_cache.shape[1]
        rep = Hq // Hkv
        q = (lambda x, *d: x.transpose(*d))((x @ wq).reshape(B, Sq, Hq, Dh), 0, 2, 1, 3)
        k = jnp.repeat(k_cache, rep, axis=1)
        v = jnp.repeat(v_cache, rep, axis=1)
        scores = jnp.einsum("bhqd,bhkd->bhqk", q, k) * (Dh ** -0.5)
        p = _softmax(scores, axis=-1)
        o = jnp.einsum("bhqk,bhkd->bhqd", p, v)
        return (lambda x, *d: x.transpose(*d))(o, 0, 2, 1, 3).reshape(B, Sq, Hq * Dh) @ wo

    def _B_ref(x, k_cache, v_cache, wq, wo):
        B, Sq, D = x.shape
        H, Dh = 32, 128
        q = (lambda x, *d: x.transpose(*d))((x @ wq).reshape(B, Sq, H, Dh), 0, 2, 1, 3)
        scores = jnp.einsum("bhqd,bhkd->bhqk", q, k_cache) * (Dh ** -0.5)
        p = _softmax(scores, axis=-1)
        o = jnp.einsum("bhqk,bhkd->bhqd", p, v_cache)
        return (lambda x, *d: x.transpose(*d))(o, 0, 2, 1, 3).reshape(B, Sq, H * Dh) @ wo

    a = _A_ref(A_x, A_k_cache, A_v_cache, A_wq, A_wo)
    b = _B_ref(B_x, B_k_cache, B_v_cache, B_wq, B_wo)
    return jnp.concatenate([a, b], axis=-1)
```

```python
import math

import jax
import jax.numpy as jnp
from jax import lax
import jax.experimental.pallas as pl
import jax.experimental.pallas.tpu as pltpu

BF16 = jnp.bfloat16
F32 = jnp.float32

BATCH, SQ, D = 16, 32, 512
SK, DH = 512, 128
ROWS = BATCH * SQ
GROUPS = 8
GCOLS = 4 * DH
UNITS = 5
KV_ROWS = 128
W_ROWS = 32

Q_SCALE = DH ** -0.5 * math.log2(math.e)

SKEW_A, SKEW_B = 1, 4
PROJ_PARTS = 4

SEM_IN, SEM_OUT, SEM_WO, SEM_K = 0, 1, 2, 3
SEM_V = SEM_K + 4 * UNITS
NUM_SEMS = SEM_V + 4 * UNITS


def _group_stream():
    def unit(kind, u):
        return [(kind, u, t, c, b) for t in range(4) for c in range(SK // KV_ROWS) for b in range(4)]

    wo = [("wo", i, (n % 4) * 4 + n // 4) for n in range(GCOLS // W_ROWS) for i in range(2)]
    v_last = unit("v", UNITS - 1)
    q0 = [d for u in range(UNITS) for d in unit("k", u)] + v_last[32::2]
    q1 = unit("v", 0) + wo + [d for u in range(1, UNITS - 1) for d in unit("v", u)] + v_last[:32] + v_last[33::2]
    assert len(q0) == len(q1)
    return list(zip(q0, q1))


STREAM = _group_stream()
PLAN = (48, 48, 24, 64, 24, 24, 52, 52)
ISSUED = [sum(PLAN[:i]) for i in range(len(PLAN) + 1)]


def _check_schedule():
    def span(pred):
        pos = [n for n, pair in enumerate(STREAM) for d in pair if pred(d)]
        return min(pos), max(pos) + 1

    def unit(u):
        return span(lambda d: d[0] != "wo" and d[1] == u)

    assert ISSUED[-1] == len(STREAM)
    assert unit(0)[1] <= ISSUED[3] and span(lambda d: d[0] == "wo")[1] <= ISSUED[4]
    assert unit(1)[1] <= ISSUED[6] and unit(2)[1] <= ISSUED[7]
    assert unit(3)[0] >= ISSUED[1] and unit(4)[0] >= ISSUED[2]


_check_schedule()


def _chunk(i, n):
    return pl.ds(i * n if isinstance(i, int) else pl.multiple_of(i * n, n), n)


def _scores(q, k):
    s = lax.dot_general(q, k, (((1,), (1,)), ((), ())), preferred_element_type=F32)
    p = jnp.exp2(s - jnp.max(s, axis=-1, keepdims=True))
    return p.astype(BF16), 1.0 / jnp.sum(p, axis=-1, keepdims=True)


def _values(scores, v):
    p, inv_sum = scores
    return (jnp.dot(p, v, preferred_element_type=F32) * inv_sum).astype(BF16)


def _kernel(ax, ak, av, awq, awo, bx, bk, bv, bwq, bwo, out,
            x_v, kv_v, wq_v, wo_v, q_v, o_v, acc_v, out_v, sem):
    def start(g, desc, queue):
        if desc[0] == "wo":
            _, i, n = desc
            rows = _chunk(g * (GCOLS // W_ROWS) + n, W_ROWS)
            src, dst, s = (awo, bwo)[i].at[rows], wo_v.at[i, rows], SEM_WO
        else:
            kind, u, t, c, b = desc
            i = int(kind == "v")
            rows = _chunk(c, KV_ROWS)
            if u == 0:
                src = (ak, av)[i].at[t * 4 + b, g, rows]
            else:
                src = (bk, bv)[i].at[(u - 1) * 4 + b, g * 4 + t, rows]
            dst, s = kv_v.at[u, i, t, b, rows], (SEM_K, SEM_V)[i] + u * 4 + t
        pltpu.make_async_copy(src, dst, sem.at[s]).start(priority=queue)

    def issue(g, lo, hi):
        for pair in STREAM[lo:hi]:
            for queue, desc in enumerate(pair):
                start(g, desc, queue)

    def issuer(g, block, parts):
        lo, n = ISSUED[block], PLAN[block]
        return lambda part: issue(g, lo + n * part // parts, lo + n * (part + 1) // parts)

    def wait(buf, s):
        pltpu.make_async_copy(buf, buf, sem.at[s]).wait()

    def wait_k(u, t):
        wait(kv_v.at[u, 0, t], SEM_K + u * 4 + t)

    def wait_v(u, t):
        wait(kv_v.at[u, 1, t], SEM_V + u * 4 + t)

    def wait_unit(u):
        for t in range(4):
            wait_k(u, t)
            wait_v(u, t)

    def q_proj(g, i, issue_part):
        for part in range(PROJ_PARTS):
            issue_part(part)
            rows = _chunk(part, ROWS // PROJ_PARTS)
            q = jnp.dot(x_v[i, rows], wq_v[i, :, _chunk(g, GCOLS)], preferred_element_type=F32)
            q_v[i, rows] = (q * Q_SCALE).astype(BF16)

    def attention_a(issue_part):
        wait_unit(0)
        scores = {}
        for step in range(BATCH + SKEW_A):
            if step < BATCH:
                issue_part(step)
                q = jnp.concatenate([q_v[0, _chunk(step, SQ), _chunk(r, DH)] for r in range(4)], axis=0)
                scores[step] = _scores(q, kv_v[0, 0, step // 4, step % 4])
            if step >= SKEW_A:
                b = step - SKEW_A
                o = _values(scores.pop(b), kv_v[0, 1, b // 4, b % 4])
                for r in range(4):
                    o_v[0, _chunk(b, SQ), _chunk(r, DH)] = o[r * SQ:(r + 1) * SQ]

    def out_proj_a(g, issue_part):
        wait(wo_v.at[:, _chunk(g, GCOLS)], SEM_WO)
        for part in range(PROJ_PARTS):
            issue_part(part)
            rows = _chunk(part, ROWS // PROJ_PARTS)
            acc_v[0, rows] += jnp.dot(o_v[0, rows], wo_v[0, _chunk(g, GCOLS)], preferred_element_type=F32)

    def attention_b(g, u, issue_part):
        wait_unit(u)
        scores = {}
        for step in range(16 + SKEW_B):
            if step < 16:
                issue_part(step)
                h, b = divmod(step, 4)
                scores[step] = _scores(q_v[1, _chunk((u - 1) * 4 + b, SQ), _chunk(h, DH)], kv_v[u, 0, h, b])
            if step >= SKEW_B:
                h, b = divmod(step - SKEW_B, 4)
                o_v[1, _chunk((u - 1) * 4 + b, SQ), _chunk(h, DH)] = _values(scores.pop(step - SKEW_B), kv_v[u, 1, h, b])
        rows = _chunk(u - 1, 4 * SQ)
        acc_v[1, rows] += jnp.dot(o_v[1, rows], wo_v[1, _chunk(g, GCOLS)], preferred_element_type=F32)

    def write_out(i, row0, nrows):
        for n in range(nrows // W_ROWS):
            rows = pl.ds(row0 + n * W_ROWS, W_ROWS)
            pltpu.make_async_copy(out_v.at[i, rows], out.at[rows, _chunk(i, D)], sem.at[SEM_OUT]).start(priority=n % 2)

    def finish(i, row0, nrows):
        rows = pl.ds(row0, nrows)
        out_v[i, rows] = acc_v[i, rows].astype(BF16)
        write_out(i, row0, nrows)

    @pl.loop(0, 4)
    def _(c):
        for n in range(4):
            rows = _chunk(n * 4 + c, W_ROWS)
            for i, ref in enumerate((ax, bx)):
                pltpu.make_async_copy(ref.at[rows], x_v.at[i, rows], sem.at[SEM_IN]).start(priority=i)

    @pl.loop(0, 16)
    def _(c):
        for n in range(8):
            rows, cols = _chunk(n * 8 + (c >> 1), 8), _chunk(c & 1, 2048)
            for i, ref in enumerate((awq, bwq)):
                pltpu.make_async_copy(ref.at[rows, cols], wq_v.at[i, rows, cols], sem.at[SEM_IN]).start(priority=i)

    @pl.loop(0, GROUPS)
    def _(g):
        @pl.when(g == 0)
        def _():
            issue(g, 0, ISSUED[2])
            acc_v[...] = jnp.zeros(acc_v.shape, F32)
            wait(x_v, SEM_IN)
            wait(wq_v, SEM_IN)

        @pl.when(g > 0)
        def _():
            attention_b(g - 1, 3, issuer(g, 0, 16))
            attention_b(g - 1, 4, issuer(g, 1, 16))

        q_proj(g, 0, issuer(g, 2, PROJ_PARTS))
        attention_a(issuer(g, 3, BATCH))
        out_proj_a(g, issuer(g, 4, PROJ_PARTS))
        pl.when(g == GROUPS - 1)(lambda: finish(0, 0, ROWS))
        q_proj(g, 1, issuer(g, 5, PROJ_PARTS))
        attention_b(g, 1, issuer(g, 6, 16))
        pl.when(g == GROUPS - 1)(lambda: finish(1, 0, 4 * SQ))
        attention_b(g, 2, issuer(g, 7, 16))

    g = GROUPS - 1
    finish(1, 4 * SQ, 4 * SQ)
    attention_b(g, 3, lambda part: None)
    finish(1, 8 * SQ, 4 * SQ)

    u = UNITS - 1
    for h in range(4):
        wait_k(u, h)
    scores = {(h, b): _scores(q_v[1, _chunk(12 + b, SQ), _chunk(h, DH)], kv_v[u, 0, h, b])
              for h in range(4) for b in range(4)}
    rows = _chunk(3, 4 * SQ)
    for half in range(2):
        heads = (2 * half, 2 * half + 1)
        for h in heads:
            wait_v(u, h)
        o = jnp.concatenate(
            [jnp.concatenate([_values(scores[h, b], kv_v[u, 1, h, b]) for h in heads], axis=1) for b in range(4)],
            axis=0)
        y = acc_v[1, rows] + jnp.dot(o, wo_v[1, _chunk(2 * g + half, 2 * DH)], preferred_element_type=F32)
        if half == 0:
            acc_v[1, rows] = y
        else:
            out_v[1, rows] = y.astype(BF16)
    write_out(1, 12 * SQ, 4 * SQ)
    wait(out_v, SEM_OUT)


@jax.jit
def pallas_concat_heads__gqa_block_cached__mha_block_cached__near_ridge_kernel(
    A_x: jax.Array,
    A_k_cache: jax.Array,
    A_v_cache: jax.Array,
    A_wq: jax.Array,
    A_wo: jax.Array,
    B_x: jax.Array,
    B_k_cache: jax.Array,
    B_v_cache: jax.Array,
    B_wq: jax.Array,
    B_wo: jax.Array,
):
    out = pl.pallas_call(
        _kernel,
        in_specs=[pl.BlockSpec(memory_space=pltpu.HBM)] * 10,
        out_specs=pl.BlockSpec(memory_space=pltpu.HBM),
        out_shape=jax.ShapeDtypeStruct((ROWS, 2 * D), BF16),
        scratch_shapes=[
            pltpu.VMEM((2, ROWS, D), BF16),
            pltpu.VMEM((UNITS, 2, 4, 4, SK, DH), BF16),
            pltpu.VMEM((2, D, GROUPS * GCOLS), BF16),
            pltpu.VMEM((2, GROUPS * GCOLS, D), BF16),
            pltpu.VMEM((2, ROWS, GCOLS), BF16),
            pltpu.VMEM((2, ROWS, GCOLS), BF16),
            pltpu.VMEM((2, ROWS, D), F32),
            pltpu.VMEM((2, ROWS, D), BF16),
            pltpu.SemaphoreType.DMA((NUM_SEMS,)),
        ],
        compiler_params=pltpu.CompilerParams(
            vmem_limit_bytes=64 * 2**20,
            disable_bounds_checks=True,
            disable_semaphore_checks=True,
        ),
    )(
        A_x.reshape(ROWS, D), A_k_cache, A_v_cache, A_wq, A_wo,
        B_x.reshape(ROWS, D), B_k_cache, B_v_cache, B_wq, B_wo,
    )
    return out.reshape(BATCH, SQ, 2 * D)
```

```python
import itertools
import math

import jax
import jax.numpy as jnp
from jax import lax
import jax.experimental.pallas as pl
import jax.experimental.pallas.tpu as pltpu

BF16 = jnp.bfloat16
F32 = jnp.float32

BATCH, SQ, D = 16, 32, 512
SK, DH = 512, 128
ROWS = BATCH * SQ
GROUPS = 8
GCOLS = 4 * DH
UNITS = 5
KV_ROWS = 128
W_ROWS = 32
GQA, MHA = 0, 1

Q_SCALE = DH ** -0.5 * math.log2(math.e)

SKEW_GQA, SKEW_MHA = 1, 4

SEM_X, SEM_WQ, SEM_OUT, SEM_WO, SEM_K = 0, 1, 2, 3, 5
SEM_V = SEM_K + UNITS
NUM_SEMS = SEM_V + UNITS - 1 + 4


def _group_stream():
    def unit(kind, u):
        return [(kind, u, b, h, c) for c, b, h in itertools.product(range(SK // KV_ROWS), range(4), range(4))]

    def merge(a, b):
        keyed = [((n + 0.5) / len(a), 0, d) for n, d in enumerate(a)]
        keyed += [((n + 0.5) / len(b), 1, d) for n, d in enumerate(b)]
        return [d for _, _, d in sorted(keyed, key=lambda t: t[:2])]

    wo = [[("wo", i, r, n) for n in range(DH // W_ROWS) for r in range(4)] for i in (GQA, MHA)]
    v_last = sorted(unit("v", UNITS - 1), key=lambda d: d[2])
    lead = 10
    q0 = merge(unit("k", 0), wo[GQA][:-lead])
    q0 += [d for u in range(1, UNITS) for d in unit("k", u)] + v_last[:lead]
    q1 = merge(unit("v", 0), wo[MHA] + wo[GQA][-lead:])
    q1 += [d for u in range(1, UNITS - 1) for d in unit("v", u)] + v_last[lead:]
    assert len(q0) == len(q1)
    return list(zip(q0, q1))


STREAM = _group_stream()

PREV_3, PREV_4, Q_GQA, ATT_GQA, OUT_GQA, Q_MHA, ATT_1, ATT_2, REST = range(9)
PLAN = (48, 48, 24, 64, 24, 24, 52, 20, 32)
ISSUED = [sum(PLAN[:i]) for i in range(len(PLAN) + 1)]


def _check_schedule():
    def span(pick):
        pos = [n for n, pair in enumerate(STREAM) for d in pair if pick(d)]
        return min(pos), max(pos) + 1

    unit = [span(lambda d, u=u: d[0] != "wo" and d[1] == u) for u in range(UNITS)]
    assert ISSUED[-1] == len(STREAM)
    assert unit[0][1] <= ISSUED[ATT_GQA] and span(lambda d: d[0] == "wo")[1] <= ISSUED[OUT_GQA]
    assert unit[1][1] <= ISSUED[ATT_1] and unit[2][1] <= ISSUED[ATT_2] and unit[3][1] <= ISSUED[REST]
    assert unit[3][0] >= ISSUED[PREV_3 + 1] and unit[4][0] >= ISSUED[PREV_4 + 1]


_check_schedule()


def _chunk(i, n):
    return pl.ds(i * n if isinstance(i, int) else pl.multiple_of(i * n, n), n)


def _head(branch, g, r):
    return 4 * g + r if branch == GQA else g + GROUPS * r


def _scores(q, k):
    s = lax.dot_general(q, k, (((1,), (1,)), ((), ())), preferred_element_type=F32)
    p = jnp.exp2(s - jnp.max(s, axis=-1, keepdims=True))
    return p.astype(BF16), 1.0 / jnp.sum(p, axis=-1, keepdims=True)


def _values(scores, v):
    p, inv_sum = scores
    return (jnp.dot(p, v, preferred_element_type=F32) * inv_sum).astype(BF16)


def _kernel(ax, ak, av, awq, awo, bx, bk, bv, bwq, bwo, out,
            x_v, kv_v, wq_v, wo_v, q_v, o_v, acc_v, out_v, sem):
    def start(g, desc, queue):
        if desc[0] == "wo":
            _, i, r, n = desc
            src = (awo, bwo)[i].at[_chunk(_head(i, g, r) * (DH // W_ROWS) + n, W_ROWS)]
            dst, s = wo_v.at[i, g, _chunk(r * (DH // W_ROWS) + n, W_ROWS)], SEM_WO + i
        else:
            kind, u, b, h, c = desc
            i = int(kind == "v")
            rows = _chunk(c, KV_ROWS)
            if u == 0:
                src = (ak, av)[i].at[4 * b + h, g, rows]
            else:
                src = (bk, bv)[i].at[4 * (u - 1) + b, _head(MHA, g, h), rows]
            dst, s = kv_v.at[u, i, b, h, rows], (SEM_K, SEM_V)[i] + u
            if kind == "v" and u == UNITS - 1:
                s += b
        pltpu.make_async_copy(src, dst, sem.at[s]).start(priority=queue)

    def issue(g, stage, part=0, parts=1):
        lo, n = ISSUED[stage], PLAN[stage]
        for pair in STREAM[lo + n * part // parts:lo + n * (part + 1) // parts]:
            for queue, desc in enumerate(pair):
                start(g, desc, queue)

    def wait(buf, s):
        pltpu.make_async_copy(buf, buf, sem.at[s]).wait()

    def wait_unit(u):
        wait(kv_v.at[u, 0], SEM_K + u)
        if u == UNITS - 1:
            for b in range(4):
                wait(kv_v.at[u, 1, b], SEM_V + u + b)
        else:
            wait(kv_v.at[u, 1], SEM_V + u)

    def q_proj(g, i):
        w = jnp.concatenate([wq_v[i, :, _chunk(_head(i, g, r), DH)] for r in range(4)], axis=1)
        q_v[i] = (jnp.dot(x_v[i], w, preferred_element_type=F32) * Q_SCALE).astype(BF16)

    def attention_gqa(g):
        wait_unit(0)
        scores = {}
        for step in range(BATCH + SKEW_GQA):
            if step < BATCH:
                issue(g, ATT_GQA, step, BATCH)
                q = jnp.concatenate([q_v[GQA, _chunk(step, SQ), _chunk(r, DH)] for r in range(4)], axis=0)
                scores[step] = _scores(q, kv_v[0, 0, step // 4, step % 4])
            if step >= SKEW_GQA:
                b = step - SKEW_GQA
                o = _values(scores.pop(b), kv_v[0, 1, b // 4, b % 4])
                for r in range(4):
                    o_v[GQA, _chunk(b, SQ), _chunk(r, DH)] = o[r * SQ:(r + 1) * SQ]

    def scores_mha(u, b, h):
        return _scores(q_v[MHA, _chunk(4 * (u - 1) + b, SQ), _chunk(h, DH)], kv_v[u, 0, b, h])

    def attention_mha(g, u, issue_g, stage):
        wait_unit(u)
        scores = {}
        for step in range(16 + SKEW_MHA):
            if step < 16:
                issue(issue_g, stage, step, 16)
                scores[step] = scores_mha(u, *divmod(step, 4))
            if step >= SKEW_MHA:
                b, h = divmod(step - SKEW_MHA, 4)
                o = _values(scores.pop(step - SKEW_MHA), kv_v[u, 1, b, h])
                o_v[MHA, _chunk(4 * (u - 1) + b, SQ), _chunk(h, DH)] = o
        rows = _chunk(u - 1, 4 * SQ)
        acc_v[MHA, rows] += jnp.dot(o_v[MHA, rows], wo_v[MHA, g], preferred_element_type=F32)

    @pl.loop(0, 4)
    def _(c):
        for n in range(4):
            rows = _chunk(4 * n + c, W_ROWS)
            for i, ref in enumerate((ax, bx)):
                pltpu.make_async_copy(ref.at[rows], x_v.at[i, rows], sem.at[SEM_X]).start(priority=i)

    @pl.loop(0, 16)
    def _(c):
        for n in range(8):
            rows, cols = _chunk(8 * n + (c >> 1), 8), _chunk(c & 1, GROUPS * GCOLS // 2)
            for i, ref in enumerate((awq, bwq)):
                pltpu.make_async_copy(ref.at[rows, cols], wq_v.at[i, rows, cols], sem.at[SEM_WQ]).start(priority=i)

    @pl.loop(0, GROUPS)
    def _(g):
        @pl.when(g == 0)
        def _():
            issue(g, PREV_3)
            issue(g, PREV_4)
            acc_v[...] = jnp.zeros(acc_v.shape, F32)
            wait(x_v, SEM_X)
            wait(wq_v, SEM_WQ)

        @pl.when(g > 0)
        def _():
            issue(g - 1, REST)
            attention_mha(g - 1, 3, g, PREV_3)
            attention_mha(g - 1, 4, g, PREV_4)

        issue(g, Q_GQA)
        q_proj(g, GQA)
        attention_gqa(g)
        wait(wo_v.at[GQA, g], SEM_WO + GQA)
        issue(g, OUT_GQA)
        acc_v[GQA] += jnp.dot(o_v[GQA], wo_v[GQA, g], preferred_element_type=F32)
        wait(wo_v.at[MHA, g], SEM_WO + MHA)
        issue(g, Q_MHA)
        q_proj(g, MHA)
        attention_mha(g, 1, g, ATT_1)
        attention_mha(g, 2, g, ATT_2)

    g = GROUPS - 1

    def finish_mha(u, scores, batches):
        rows = pl.ds((4 * (u - 1) + batches[0]) * SQ, len(batches) * SQ)
        o = jnp.concatenate(
            [jnp.concatenate([_values(scores[b, h], kv_v[u, 1, b, h]) for h in range(4)], axis=1) for b in batches],
            axis=0)
        y = acc_v[MHA, rows] + jnp.dot(o, wo_v[MHA, g], preferred_element_type=F32)
        out_v[rows, _chunk(MHA, D)] = y.astype(BF16)

    def write(batches):
        for b in batches:
            rows = _chunk(b, SQ)
            pltpu.make_async_copy(out_v.at[rows], out.at[rows], sem.at[SEM_OUT]).start(priority=b % 2)

    wait(kv_v.at[3, 0], SEM_K + 3)
    scores = {}
    for step in range(16):
        issue(g, REST, step, 16)
        scores[divmod(step, 4)] = scores_mha(3, *divmod(step, 4))
    out_v[:, _chunk(GQA, D)] = acc_v[GQA].astype(BF16)
    out_v[_chunk(0, 8 * SQ), _chunk(MHA, D)] = acc_v[MHA, _chunk(0, 8 * SQ)].astype(BF16)
    wait(kv_v.at[3, 1], SEM_V + 3)
    finish_mha(3, scores, (0, 1, 2, 3))

    wait(kv_v.at[4, 0], SEM_K + 4)
    scores = {(b, h): scores_mha(4, b, h) for b in range(4) for h in range(4)}
    wait(kv_v.at[4, 1, 0], SEM_V + 4)
    wait(kv_v.at[4, 1, 1], SEM_V + 5)
    finish_mha(4, scores, (0, 1))
    wait(kv_v.at[4, 1, 2], SEM_V + 6)
    write(range(14))
    finish_mha(4, scores, (2,))
    write([14])
    wait(kv_v.at[4, 1, 3], SEM_V + 7)
    finish_mha(4, scores, (3,))
    write([15])
    pltpu.make_async_copy(out_v, out, sem.at[SEM_OUT]).wait()


@jax.jit
def pallas_concat_heads__gqa_block_cached__mha_block_cached__near_ridge_kernel(
    A_x: jax.Array,
    A_k_cache: jax.Array,
    A_v_cache: jax.Array,
    A_wq: jax.Array,
    A_wo: jax.Array,
    B_x: jax.Array,
    B_k_cache: jax.Array,
    B_v_cache: jax.Array,
    B_wq: jax.Array,
    B_wo: jax.Array,
):
    out = pl.pallas_call(
        _kernel,
        in_specs=[pl.BlockSpec(memory_space=pltpu.HBM)] * 10,
        out_specs=pl.BlockSpec(memory_space=pltpu.HBM),
        out_shape=jax.ShapeDtypeStruct((ROWS, 2 * D), BF16),
        scratch_shapes=[
            pltpu.VMEM((2, ROWS, D), BF16),
            pltpu.VMEM((UNITS, 2, 4, 4, SK, DH), BF16),
            pltpu.VMEM((2, D, GROUPS * GCOLS), BF16),
            pltpu.VMEM((2, GROUPS, GCOLS, D), BF16),
            pltpu.VMEM((2, ROWS, GCOLS), BF16),
            pltpu.VMEM((2, ROWS, GCOLS), BF16),
            pltpu.VMEM((2, ROWS, D), F32),
            pltpu.VMEM((ROWS, 2 * D), BF16),
            pltpu.SemaphoreType.DMA((NUM_SEMS,)),
        ],
        compiler_params=pltpu.CompilerParams(
            vmem_limit_bytes=64 * 2**20,
            disable_semaphore_checks=True,
        ),
    )(
        A_x.reshape(ROWS, D), A_k_cache, A_v_cache, A_wq, A_wo,
        B_x.reshape(ROWS, D), B_k_cache, B_v_cache, B_wq, B_wo,
    )
    return out.reshape(BATCH, SQ, 2 * D)
```

```python
import itertools
import math

import jax
import jax.numpy as jnp
from jax import lax
import jax.experimental.pallas as pl
import jax.experimental.pallas.tpu as pltpu

BF16 = jnp.bfloat16
F32 = jnp.float32

BATCH, SQ, D = 16, 32, 512
SK, DH = 512, 128
ROWS = BATCH * SQ
GROUPS = 8
GCOLS = 4 * DH
UNITS = 5
KV_ROWS = 128
W_ROWS = 32
GQA, MHA = 0, 1

Q_SCALE = DH ** -0.5 * math.log2(math.e)

SKEW_GQA, SKEW_MHA = 1, 4

SEM_X, SEM_WQ, SEM_OUT, SEM_WO, SEM_K = 0, 1, 2, 3, 5
SEM_V = SEM_K + UNITS
NUM_SEMS = SEM_V + UNITS - 1 + 4


def _group_stream():
    def unit(kind, u):
        return [(kind, u, b, h, c) for c, b, h in itertools.product(range(SK // KV_ROWS), range(4), range(4))]

    def merge(a, b):
        keyed = [((n + 0.5) / len(a), 0, d) for n, d in enumerate(a)]
        keyed += [((n + 0.5) / len(b), 1, d) for n, d in enumerate(b)]
        return [d for _, _, d in sorted(keyed, key=lambda t: t[:2])]

    wo = [[("wo", i, r, n) for n in range(DH // W_ROWS) for r in range(4)] for i in (GQA, MHA)]
    v_last = sorted(unit("v", UNITS - 1), key=lambda d: d[2])
    lead = 12
    q0 = merge(unit("k", 0), wo[GQA][:-lead])
    q0 += [d for u in range(1, UNITS) for d in unit("k", u)] + v_last[:lead]
    q1 = merge(unit("v", 0), wo[MHA] + wo[GQA][-lead:])
    q1 += [d for u in range(1, UNITS - 1) for d in unit("v", u)] + v_last[lead:]
    assert len(q0) == len(q1)
    return list(zip(q0, q1))


STREAM = _group_stream()

PREV_3, PREV_4, Q_GQA, ATT_GQA, OUT_GQA, Q_MHA, ATT_1, ATT_2, REST = range(9)
PLAN = (48, 48, 24, 64, 24, 24, 52, 20, 32)
ISSUED = [sum(PLAN[:i]) for i in range(len(PLAN) + 1)]


def _check_schedule():
    def span(pick):
        pos = [n for n, pair in enumerate(STREAM) for d in pair if pick(d)]
        return min(pos), max(pos) + 1

    unit = [span(lambda d, u=u: d[0] != "wo" and d[1] == u) for u in range(UNITS)]
    assert ISSUED[-1] == len(STREAM)
    assert unit[0][1] <= ISSUED[ATT_GQA] and span(lambda d: d[0] == "wo")[1] <= ISSUED[OUT_GQA]
    assert unit[1][1] <= ISSUED[ATT_1] and unit[2][1] <= ISSUED[ATT_2] and unit[3][1] <= ISSUED[REST]
    assert unit[3][0] >= ISSUED[PREV_3 + 1] and unit[4][0] >= ISSUED[PREV_4 + 1]


_check_schedule()


def _chunk(i, n):
    return pl.ds(i * n if isinstance(i, int) else pl.multiple_of(i * n, n), n)


def _head(branch, g, r):
    return 4 * g + r if branch == GQA else g + GROUPS * r


def _scores(q, k):
    s = lax.dot_general(q, k, (((1,), (1,)), ((), ())), preferred_element_type=F32)
    p = jnp.exp2(s - jnp.max(s, axis=-1, keepdims=True))
    return p.astype(BF16), 1.0 / jnp.sum(p, axis=-1, keepdims=True)


def _values(scores, v):
    p, inv_sum = scores
    return (jnp.dot(p, v, preferred_element_type=F32) * inv_sum).astype(BF16)


def _kernel(ax, ak, av, awq, awo, bx, bk, bv, bwq, bwo, out,
            x_v, kv_v, wq_v, wo_v, q_v, o_v, acc_v, out_v, sem):
    def start(g, desc, queue):
        if desc[0] == "wo":
            _, i, r, n = desc
            src = (awo, bwo)[i].at[_chunk(_head(i, g, r) * (DH // W_ROWS) + n, W_ROWS)]
            dst, s = wo_v.at[i, g, _chunk(r * (DH // W_ROWS) + n, W_ROWS)], SEM_WO + i
        else:
            kind, u, b, h, c = desc
            i = int(kind == "v")
            rows = _chunk(c, KV_ROWS)
            if u == 0:
                src = (ak, av)[i].at[4 * b + h, g, rows]
            else:
                src = (bk, bv)[i].at[4 * (u - 1) + b, _head(MHA, g, h), rows]
            dst, s = kv_v.at[u, i, b, h, rows], (SEM_K, SEM_V)[i] + u
            if kind == "v" and u == UNITS - 1:
                s += b
        pltpu.make_async_copy(src, dst, sem.at[s]).start(priority=queue)

    def issue(g, stage, part=0, parts=1):
        lo, n = ISSUED[stage], PLAN[stage]
        for pair in STREAM[lo + n * part // parts:lo + n * (part + 1) // parts]:
            for queue, desc in enumerate(pair):
                start(g, desc, queue)

    def wait(buf, s):
        pltpu.make_async_copy(buf, buf, sem.at[s]).wait()

    def wait_unit(u):
        wait(kv_v.at[u, 0], SEM_K + u)
        if u == UNITS - 1:
            for b in range(4):
                wait(kv_v.at[u, 1, b], SEM_V + u + b)
        else:
            wait(kv_v.at[u, 1], SEM_V + u)

    def q_proj(g, i):
        w = jnp.concatenate([wq_v[i, :, _chunk(_head(i, g, r), DH)] for r in range(4)], axis=1)
        q_v[i] = (jnp.dot(x_v[i], w, preferred_element_type=F32) * Q_SCALE).astype(BF16)

    def attention_gqa(g):
        wait_unit(0)
        scores = {}
        for step in range(BATCH + SKEW_GQA):
            if step < BATCH:
                issue(g, ATT_GQA, step, BATCH)
                q = jnp.concatenate([q_v[GQA, _chunk(step, SQ), _chunk(r, DH)] for r in range(4)], axis=0)
                scores[step] = _scores(q, kv_v[0, 0, step // 4, step % 4])
            if step >= SKEW_GQA:
                b = step - SKEW_GQA
                o = _values(scores.pop(b), kv_v[0, 1, b // 4, b % 4])
                for r in range(4):
                    o_v[GQA, _chunk(b, SQ), _chunk(r, DH)] = o[r * SQ:(r + 1) * SQ]

    def scores_mha(u, b, h):
        return _scores(q_v[MHA, _chunk(4 * (u - 1) + b, SQ), _chunk(h, DH)], kv_v[u, 0, b, h])

    def attention_mha(g, u, issue_g, stage):
        wait_unit(u)
        scores = {}
        for step in range(16 + SKEW_MHA):
            if step < 16:
                issue(issue_g, stage, step, 16)
                scores[step] = scores_mha(u, *divmod(step, 4))
            if step >= SKEW_MHA:
                b, h = divmod(step - SKEW_MHA, 4)
                o = _values(scores.pop(step - SKEW_MHA), kv_v[u, 1, b, h])
                o_v[MHA, _chunk(4 * (u - 1) + b, SQ), _chunk(h, DH)] = o
        rows = _chunk(u - 1, 4 * SQ)
        acc_v[MHA, rows] += jnp.dot(o_v[MHA, rows], wo_v[MHA, g], preferred_element_type=F32)

    for n in range(128):
        rows, cols = _chunk(8 * (n % 8) + n // 16, 8), _chunk(n // 8 % 2, GROUPS * GCOLS // 2)
        for i, ref in enumerate((awq, bwq)):
            pltpu.make_async_copy(ref.at[rows, cols], wq_v.at[i, rows, cols], sem.at[SEM_WQ]).start(priority=i)
        if n % 8 == 7:
            rows = _chunk(n // 8, W_ROWS)
            for i, ref in enumerate((ax, bx)):
                pltpu.make_async_copy(ref.at[rows], x_v.at[i, rows], sem.at[SEM_X]).start(priority=i)

    @pl.loop(0, GROUPS)
    def _(g):
        @pl.when(g == 0)
        def _():
            issue(g, PREV_3)
            issue(g, PREV_4)
            acc_v[...] = jnp.zeros(acc_v.shape, F32)
            wait(x_v, SEM_X)
            wait(wq_v, SEM_WQ)

        @pl.when(g > 0)
        def _():
            issue(g - 1, REST)
            attention_mha(g - 1, 3, g, PREV_3)
            attention_mha(g - 1, 4, g, PREV_4)

        issue(g, Q_GQA)
        q_proj(g, GQA)
        attention_gqa(g)
        wait(wo_v.at[GQA, g], SEM_WO + GQA)
        issue(g, OUT_GQA)
        acc_v[GQA] += jnp.dot(o_v[GQA], wo_v[GQA, g], preferred_element_type=F32)
        wait(wo_v.at[MHA, g], SEM_WO + MHA)
        issue(g, Q_MHA)
        q_proj(g, MHA)
        attention_mha(g, 1, g, ATT_1)
        attention_mha(g, 2, g, ATT_2)

    g = GROUPS - 1

    def finish_mha(u, scores, batches):
        rows = pl.ds((4 * (u - 1) + batches[0]) * SQ, len(batches) * SQ)
        o = jnp.concatenate(
            [jnp.concatenate([_values(scores[b, h], kv_v[u, 1, b, h]) for h in range(4)], axis=1) for b in batches],
            axis=0)
        y = acc_v[MHA, rows] + jnp.dot(o, wo_v[MHA, g], preferred_element_type=F32)
        out_v[rows, _chunk(MHA, D)] = y.astype(BF16)

    def write(batches):
        for b in batches:
            rows = _chunk(b, SQ)
            pltpu.make_async_copy(out_v.at[rows], out.at[rows], sem.at[SEM_OUT]).start(priority=b % 2)

    wait(kv_v.at[3, 0], SEM_K + 3)
    scores = {}
    for step in range(16):
        issue(g, REST, step, 16)
        scores[divmod(step, 4)] = scores_mha(3, *divmod(step, 4))
    out_v[:, _chunk(GQA, D)] = acc_v[GQA].astype(BF16)
    out_v[_chunk(0, 8 * SQ), _chunk(MHA, D)] = acc_v[MHA, _chunk(0, 8 * SQ)].astype(BF16)
    wait(kv_v.at[3, 1], SEM_V + 3)
    finish_mha(3, scores, (0, 1, 2, 3))

    wait(kv_v.at[4, 0], SEM_K + 4)
    scores = {(b, h): scores_mha(4, b, h) for b in range(4) for h in range(4)}
    wait(kv_v.at[4, 1, 0], SEM_V + 4)
    wait(kv_v.at[4, 1, 1], SEM_V + 5)
    finish_mha(4, scores, (0, 1))
    wait(kv_v.at[4, 1, 2], SEM_V + 6)
    write(range(14))
    finish_mha(4, scores, (2,))
    write([14])
    wait(kv_v.at[4, 1, 3], SEM_V + 7)
    finish_mha(4, scores, (3,))
    write([15])
    pltpu.make_async_copy(out_v, out, sem.at[SEM_OUT]).wait()


@jax.jit
def pallas_concat_heads__gqa_block_cached__mha_block_cached__near_ridge_kernel(
    A_x: jax.Array,
    A_k_cache: jax.Array,
    A_v_cache: jax.Array,
    A_wq: jax.Array,
    A_wo: jax.Array,
    B_x: jax.Array,
    B_k_cache: jax.Array,
    B_v_cache: jax.Array,
    B_wq: jax.Array,
    B_wo: jax.Array,
):
    out = pl.pallas_call(
        _kernel,
        in_specs=[pl.BlockSpec(memory_space=pltpu.HBM)] * 10,
        out_specs=pl.BlockSpec(memory_space=pltpu.HBM),
        out_shape=jax.ShapeDtypeStruct((ROWS, 2 * D), BF16),
        scratch_shapes=[
            pltpu.VMEM((2, ROWS, D), BF16),
            pltpu.VMEM((UNITS, 2, 4, 4, SK, DH), BF16),
            pltpu.VMEM((2, D, GROUPS * GCOLS), BF16),
            pltpu.VMEM((2, GROUPS, GCOLS, D), BF16),
            pltpu.VMEM((2, ROWS, GCOLS), BF16),
            pltpu.VMEM((2, ROWS, GCOLS), BF16),
            pltpu.VMEM((2, ROWS, D), F32),
            pltpu.VMEM((ROWS, 2 * D), BF16),
            pltpu.SemaphoreType.DMA((NUM_SEMS,)),
        ],
        compiler_params=pltpu.CompilerParams(
            vmem_limit_bytes=64 * 2**20,
            disable_semaphore_checks=True,
        ),
    )(
        A_x.reshape(ROWS, D), A_k_cache, A_v_cache, A_wq, A_wo,
        B_x.reshape(ROWS, D), B_k_cache, B_v_cache, B_wq, B_wo,
    )
    return out.reshape(BATCH, SQ, 2 * D)
```
